```python
import jax
import jax.numpy as jnp

def _softmax(x, axis=-1):
    return jax.nn.softmax(x, axis=axis)
def _gelu(x):
    return jax.nn.gelu(x, approximate=True)
def _silu(x):
    return jax.nn.silu(x)
def _sigmoid(x):
    return jax.nn.sigmoid(x)
def _layernorm(x, axis=-1, eps=1e-5):
    m = jnp.mean(x, axis=axis, keepdims=True)
    v = jnp.var(x, axis=axis, keepdims=True)
    return (x - m) / jnp.sqrt(v + eps)
def _scatter_add(tgt, idx, src, axis=0):
    return tgt.at[idx].add(src)
def _segment_sum(src, seg, n):
    return jax.ops.segment_sum(src, seg, n)
class _Rng:
    def __init__(self, key):
        self._k = key
    def _next(self):
        self._k, sub = jax.random.split(self._k)
        return sub
    def normal(self, shape):
        return jax.random.normal(self._next(), shape, dtype=jnp.bfloat16)
    def randint(self, lo, hi, shape):
        return jax.random.randint(self._next(), shape, lo, hi, dtype=jnp.int32)
    def uniform(self, shape, lo=0.0, hi=1.0):
        return jax.random.uniform(self._next(), shape, jnp.bfloat16, lo, hi)
    def permutation(self, n):
        return jax.random.permutation(self._next(), n)


kernel_name = 'gated_mix__sliding_block_cached__dense_activation_gelu__decode'

def setup_inputs():
    _rng = _Rng(jax.random.key(int.from_bytes(__import__("os").urandom(4), "little")))
    _w = (lambda a: (lambda t: t.astype(jnp.bfloat16) if jnp.issubdtype(t.dtype, jnp.floating) else t)(jnp.asarray(a)))
    def _A_setup():
        B, Sq, D = 1, 1, 640
        Hq, Hkv, Sk, Dh = 32, 32, 32768, 192
        assert Hq % Hkv == 0, (Hq, Hkv)
        return {
            "x": _w((lambda *s: _rng.normal(s) * 0.05)(B, Sq, D)),
            "k_cache": _w((lambda *s: _rng.normal(s) * 0.05)(B, Hkv, Sk, Dh)),
            "v_cache": _w((lambda *s: _rng.normal(s) * 0.05)(B, Hkv, Sk, Dh)),
            "wq": _w((lambda *s: _rng.normal(s) * 0.05)(D, Hq * Dh) * (D ** -0.5)),
            "wo": _w((lambda *s: _rng.normal(s) * 0.05)(Hq * Dh, D) * ((Hq * Dh) ** -0.5)),
        }
    _A_in = _A_setup()

    def _B_setup():
        B, S, D, F = 1, 1, 640, 1536
        return {
            "x": _w((lambda *s: _rng.normal(s) * 0.05)(B, S, D)),
            "w1": _w((lambda *s: _rng.normal(s) * 0.05)(D, F) * (D ** -0.5)),
            "b1": _w((lambda *s: _rng.normal(s) * 0.05)(F) * 0.01),
            "w2": _w((lambda *s: _rng.normal(s) * 0.05)(F, D) * (F ** -0.5)),
            "b2": _w((lambda *s: _rng.normal(s) * 0.05)(D) * 0.01),
        }
    _B_in = _B_setup()

    return {
        "A_x": _A_in["x"],
        "A_k_cache": _A_in["k_cache"],
        "A_v_cache": _A_in["v_cache"],
        "A_wq": _A_in["wq"],
        "A_wo": _A_in["wo"],
        "B_x": _B_in["x"],
        "B_w1": _B_in["w1"],
        "B_b1": _B_in["b1"],
        "B_w2": _B_in["w2"],
        "B_b2": _B_in["b2"],
        "gate_w": _w((lambda *s: _rng.normal(s) * 0.05)(640)),
    }

def reference(A_x, A_k_cache, A_v_cache, A_wq, A_wo, B_x, B_w1, B_b1, B_w2, B_b2, gate_w):
    def _A_ref(x, k_cache, v_cache, wq, wo):
        B, Sq, D = x.shape
        Hq, Dh = 32, 192
        Hkv, Sk = k_cache.shape[1], k_cache.shape[2]
        W = min(4096, max(256, Sk // 4))
        rep = Hq // Hkv
        q = (lambda x, *d: x.transpose(*d))((x @ wq).reshape(B, Sq, Hq, Dh), 0, 2, 1, 3)
        k = jnp.repeat(k_cache[:, :, Sk - W:, :], rep, axis=1)
        v = jnp.repeat(v_cache[:, :, Sk - W:, :], rep, axis=1)
        scores = jnp.einsum("bhqd,bhkd->bhqk", q, k) * (Dh ** -0.5)
        p = _softmax(scores, axis=-1)
        o = jnp.einsum("bhqk,bhkd->bhqd", p, v)
        return (lambda x, *d: x.transpose(*d))(o, 0, 2, 1, 3).reshape(B, Sq, Hq * Dh) @ wo

    def _B_ref(x, w1, b1, w2, b2):
        h = jnp.einsum("bsd,df->bsf", x, w1) + b1
        h = _gelu(h)
        return jnp.einsum("bsf,fd->bsd", h, w2) + b2

    x = A_x
    g = _sigmoid((x * gate_w).sum(-1, keepdims=True))
    a = _A_ref(x, A_k_cache, A_v_cache, A_wq, A_wo)
    b = _B_ref(x, B_w1, B_b1, B_w2, B_b2)
    return g * a + (1 - g) * b
```

```python
import jax
import jax.numpy as jnp
import jax.experimental.pallas as pl
import jax.experimental.pallas.tpu as pltpu

_HQ, _DH = 32, 192
_NS = 2
_VC = 4


@jax.jit
def pallas_gated_mix__sliding_block_cached__dense_activation_gelu__decode_kernel(
    A_x: jax.Array,
    A_k_cache: jax.Array,
    A_v_cache: jax.Array,
    A_wq: jax.Array,
    A_wo: jax.Array,
    B_x: jax.Array,
    B_w1: jax.Array,
    B_b1: jax.Array,
    B_w2: jax.Array,
    B_b2: jax.Array,
    gate_w: jax.Array,
):
    del B_x
    batch, sq, d = A_x.shape
    _, hkv, sk, dh = A_k_cache.shape
    f = B_w1.shape[1]
    assert (batch, sq) == (1, 1) and (hkv, dh) == (_HQ, _DH)
    win = min(4096, max(256, sk // 4))
    w0 = sk - win
    n_pairs = _HQ // 2
    pr = 2 * _DH
    ns, vc = _NS, _VC
    vw = win // vc
    scale = _DH ** -0.5
    f32, bf16 = jnp.float32, jnp.bfloat16

    def kernel_function(
        x_hbm, gw_hbm, b1_hbm, b2_hbm, kt_hbm, vt_hbm, wq_hbm, wo_hbm, w1_hbm, w2_hbm,
        o_ref,
        xbuf, gwbuf, b1buf, b2buf, kbuf, vbuf, wqbuf, wobuf, w1buf, w2buf,
        ksem, vsem, wqsem, wosem, fsem,
    ):
        def k_copy(j, slot):
            return pltpu.make_async_copy(
                kt_hbm.at[j, :, pl.ds(w0, win)], kbuf.at[slot], ksem.at[slot])

        def v_copy(j, slot, c):
            return pltpu.make_async_copy(
                vt_hbm.at[j, :, pl.ds(w0 + c * vw, vw)], vbuf.at[slot, c], vsem.at[slot, c])

        def wq_copy(j, slot):
            return pltpu.make_async_copy(
                wq_hbm.at[:, pl.ds(pl.multiple_of(j * pr, 128), pr)], wqbuf.at[slot], wqsem.at[slot])

        def wo_copy(j, slot):
            return pltpu.make_async_copy(
                wo_hbm.at[pl.ds(pl.multiple_of(j * pr, 128), pr), :], wobuf.at[slot], wosem.at[slot])

        x_cp, gw_cp, b1_cp, b2_cp, w1_cp, w2_cp = [
            pltpu.make_async_copy(src, dst, fsem.at[i])
            for i, (src, dst) in enumerate([
                (x_hbm, xbuf), (gw_hbm, gwbuf), (b1_hbm, b1buf),
                (b2_hbm, b2buf), (w1_hbm, w1buf), (w2_hbm, w2buf)])
        ]

        def start_k(j, slot):
            wq_copy(j, slot).start()
            k_copy(j, slot).start()

        def start_v(j, slot):
            for c in range(vc):
                v_copy(j, slot, c).start()

        for cp in (x_cp, gw_cp, b1_cp, b2_cp, w1_cp, w2_cp):
            cp.start()
        x_cp.wait()
        for s in range(ns):
            start_k(s, s)
            start_v(s, s)
            wo_copy(s, s).start()

        x = xbuf[0]
        x8 = jnp.broadcast_to(x, (8, d))

        gw_cp.wait()
        g = jax.nn.sigmoid(
            jnp.sum(x.astype(f32) * gwbuf[...].astype(f32).reshape(1, d), axis=-1, keepdims=True))
        w1_cp.wait()
        b1_cp.wait()
        h = jnp.dot(x8, w1buf[...], preferred_element_type=f32) + b1buf[...].astype(f32).reshape(1, f)
        h = jax.nn.gelu(h, approximate=True)
        w2_cp.wait()
        b2_cp.wait()
        b = (jnp.dot(h.astype(bf16), w2buf[...], preferred_element_type=f32)[0:1]
             + b2buf[...].astype(f32).reshape(1, d))
        mlp_term = (1 - g) * b

        col = jax.lax.broadcasted_iota(jnp.int32, (8, pr), 1)
        row = jax.lax.broadcasted_iota(jnp.int32, (8, pr), 0)
        own_head = (col < _DH) == (row < 4)

        def body(j, acc):
            slot = j % ns
            wq_copy(j, slot).wait()
            q = jnp.dot(x8, wqbuf[slot], preferred_element_type=f32)
            q = jnp.where(own_head, q, 0.0).astype(bf16)
            k_copy(j, slot).wait()
            s = jnp.dot(q, kbuf[slot], preferred_element_type=f32) * scale
            m = jnp.max(s, axis=-1, keepdims=True)
            p = jnp.exp(s - m)
            l = jnp.sum(p, axis=-1, keepdims=True)
            p = p.astype(bf16)

            @pl.when(j + ns < n_pairs)
            def _():
                start_k(j + ns, slot)

            o = jnp.zeros((8, pr), f32)
            for c in range(vc):
                v_copy(j, slot, c).wait()
                o = o + jax.lax.dot_general(
                    p[:, c * vw:(c + 1) * vw], vbuf[slot, c],
                    (((1,), (1,)), ((), ())), preferred_element_type=f32)
            o = jnp.where(own_head, o / l, 0.0)

            @pl.when(j + ns < n_pairs)
            def _():
                start_v(j + ns, slot)

            wo_copy(j, slot).wait()
            acc = acc + jnp.dot(o.astype(bf16), wobuf[slot], preferred_element_type=f32)

            @pl.when(j + ns < n_pairs)
            def _():
                wo_copy(j + ns, slot).start()

            return acc

        acc = jax.lax.fori_loop(0, n_pairs, body, jnp.zeros((8, d), f32))
        a = acc[0:1] + acc[4:5]
        o_ref[0] = (g * a + mlp_term).astype(o_ref.dtype)

    kt = jnp.transpose(A_k_cache, (0, 1, 3, 2)).reshape(n_pairs, pr, sk)
    vt = jnp.transpose(A_v_cache, (0, 1, 3, 2)).reshape(n_pairs, pr, sk)

    return pl.pallas_call(
        kernel_function,
        in_specs=[pl.BlockSpec(memory_space=pl.ANY) for _ in range(10)],
        out_specs=pl.BlockSpec(memory_space=pltpu.VMEM),
        out_shape=jax.ShapeDtypeStruct((batch, sq, d), A_x.dtype),
        scratch_shapes=[
            pltpu.VMEM((batch, sq, d), A_x.dtype),
            pltpu.VMEM((d,), gate_w.dtype),
            pltpu.VMEM((f,), B_b1.dtype),
            pltpu.VMEM((d,), B_b2.dtype),
            pltpu.VMEM((ns, pr, win), A_k_cache.dtype),
            pltpu.VMEM((ns, vc, pr, vw), A_v_cache.dtype),
            pltpu.VMEM((ns, d, pr), A_wq.dtype),
            pltpu.VMEM((ns, pr, d), A_wo.dtype),
            pltpu.VMEM((d, f), B_w1.dtype),
            pltpu.VMEM((f, d), B_w2.dtype),
            pltpu.SemaphoreType.DMA((ns,)),
            pltpu.SemaphoreType.DMA((ns, vc)),
            pltpu.SemaphoreType.DMA((ns,)),
            pltpu.SemaphoreType.DMA((ns,)),
            pltpu.SemaphoreType.DMA((6,)),
        ],
        compiler_params=pltpu.CompilerParams(vmem_limit_bytes=64 * 1024 * 1024),
    )(A_x, gate_w, B_b1, B_b2, kt, vt, A_wq, A_wo, B_w1, B_w2)
```

```python
import functools

import jax
import jax.numpy as jnp
import jax.experimental.pallas as pl
import jax.experimental.pallas.tpu as pltpu

_HQ, _DH = 32, 192
_PR = 2 * _DH
_LANES = 128

_WQ_PIECES = 3
_K_COLS = 128
_V_ROWS, _V_COLS = 128, 512
_MLP_PIECES = 2
_LOOKAHEAD = 13


@jax.jit
def pallas_gated_mix__sliding_block_cached__dense_activation_gelu__decode_kernel(
    A_x: jax.Array,
    A_k_cache: jax.Array,
    A_v_cache: jax.Array,
    A_wq: jax.Array,
    A_wo: jax.Array,
    B_x: jax.Array,
    B_w1: jax.Array,
    B_b1: jax.Array,
    B_w2: jax.Array,
    B_b2: jax.Array,
    gate_w: jax.Array,
):
    del B_x
    batch, sq, d = A_x.shape
    _, hkv, sk, dh = A_k_cache.shape
    f = B_w1.shape[1]
    assert (batch, sq) == (1, 1) and (hkv, dh) == (_HQ, _DH)
    win = min(4096, max(256, sk // 4))
    w0 = sk - win
    n_pairs = _HQ // 2
    scale = _DH ** -0.5
    f32, bf16 = jnp.float32, jnp.bfloat16

    wq_cols = _PR // _WQ_PIECES
    nk = win // _K_COLS
    nvr, nvc = _PR // _V_ROWS, win // _V_COLS
    fc = f // _MLP_PIECES
    pieces = ([("wq", i, 0) for i in range(_WQ_PIECES)]
              + [("k", 0, i) for i in range(nk)]
              + [("v", r, c) for r in range(nvr) for c in range(nvc)]
              + [("wo", 0, 0)])
    n_pieces = len(pieces)
    assert _LOOKAHEAD <= n_pieces

    def kernel_function(
        x_hbm, gw_hbm, b1_hbm, b2_hbm, kt_hbm, vt_hbm, wq_hbm, wo_hbm, w1_hbm, w2_hbm,
        o_ref,
        xbuf, gwbuf, b1buf, b2buf, kbuf, vbuf, wqbuf, wobuf, w1buf, w2buf,
        ksem, vsem, wqsem, wosem, vec_sem, mlp_sem,
    ):
        def copy(t, pair, slot):
            kind, r, c = pieces[t]
            if kind == "wq":
                cols = pl.ds(pl.multiple_of(pair * _PR + r * wq_cols, _LANES), wq_cols)
                return pltpu.make_async_copy(
                    wq_hbm.at[:, cols], wqbuf.at[slot, :, pl.ds(r * wq_cols, wq_cols)], wqsem.at[slot, r])
            if kind == "wo":
                rows = pl.ds(pl.multiple_of(pair * _PR, _LANES), _PR)
                return pltpu.make_async_copy(wo_hbm.at[rows, :], wobuf.at[slot], wosem.at[slot])
            if kind == "k":
                return pltpu.make_async_copy(
                    kt_hbm.at[pair, :, pl.ds(w0 + c * _K_COLS, _K_COLS)],
                    kbuf.at[slot, :, pl.ds(c * _K_COLS, _K_COLS)], ksem.at[slot, c])
            rows, cols = pl.ds(r * _V_ROWS, _V_ROWS), pl.ds(c * _V_COLS, _V_COLS)
            return pltpu.make_async_copy(
                vt_hbm.at[pair, rows, pl.ds(w0 + c * _V_COLS, _V_COLS)],
                vbuf.at[slot, rows, cols], vsem.at[slot, r * nvc + c])

        def start(t, pair, slot):
            copy(t, pair, slot).start(priority=t % 2)

        def advance(t, pair, slot, last):
            ahead, t2 = divmod(t + _LOOKAHEAD, n_pieces)
            if last and ahead:
                return
            start(t2, pair + ahead, 1 - slot if ahead else slot)

        x_cp, gw_cp, b1_cp, b2_cp = [
            pltpu.make_async_copy(src, dst, vec_sem.at[i])
            for i, (src, dst) in enumerate(
                [(x_hbm, xbuf), (gw_hbm, gwbuf), (b1_hbm, b1buf), (b2_hbm, b2buf)])
        ]
        w1_cps = [
            pltpu.make_async_copy(
                w1_hbm.at[:, pl.ds(i * fc, fc)], w1buf.at[:, pl.ds(i * fc, fc)], mlp_sem.at[0, i])
            for i in range(_MLP_PIECES)
        ]
        w2_cps = [
            pltpu.make_async_copy(
                w2_hbm.at[pl.ds(i * fc, fc), :], w2buf.at[pl.ds(i * fc, fc), :], mlp_sem.at[1, i])
            for i in range(_MLP_PIECES)
        ]
        for cp in (x_cp, gw_cp, b1_cp, b2_cp):
            cp.start()
        for i, cp in enumerate(w1_cps + w2_cps):
            cp.start(priority=i % 2)
        x_cp.wait()
        for g in range(_LOOKAHEAD):
            pair, t = divmod(g, n_pieces)
            start(t, pair, pair % 2)

        x = xbuf[0]
        x8 = jnp.broadcast_to(x, (8, d))

        gw_cp.wait()
        gate = jax.nn.sigmoid(
            jnp.sum(x.astype(f32) * gwbuf[...].astype(f32).reshape(1, d), axis=-1, keepdims=True))
        b1_cp.wait()
        for cp in w1_cps:
            cp.wait()
        h = jnp.dot(x8, w1buf[...], preferred_element_type=f32) + b1buf[...].astype(f32).reshape(1, f)
        h = jax.nn.gelu(h, approximate=True)
        b2_cp.wait()
        for cp in w2_cps:
            cp.wait()
        b = (jnp.dot(h.astype(bf16), w2buf[...], preferred_element_type=f32)[0:1]
             + b2buf[...].astype(f32).reshape(1, d))
        mlp_term = (1 - gate) * b

        col = jax.lax.broadcasted_iota(jnp.int32, (8, _PR), 1)
        row = jax.lax.broadcasted_iota(jnp.int32, (8, _PR), 0)
        own_head = (col < _DH) == (row < 4)

        def body(pair, acc, last=False):
            slot = pair % 2

            def consume(t, fn):
                copy(t, pair, slot).wait()
                out = fn()
                advance(t, pair, slot, last)
                return out

            t = 0
            qs = []
            for i in range(_WQ_PIECES):
                qs.append(consume(t, lambda: jnp.dot(
                    x8, wqbuf[slot, :, pl.ds(i * wq_cols, wq_cols)], preferred_element_type=f32)))
                t += 1
            q = jnp.where(own_head, jnp.concatenate(qs, axis=-1), 0.0).astype(bf16)

            scores = []
            for c in range(nk):
                scores.append(consume(t, lambda: jnp.dot(
                    q, kbuf[slot, :, pl.ds(c * _K_COLS, _K_COLS)], preferred_element_type=f32) * scale))
                t += 1
            m = functools.reduce(jnp.maximum, [jnp.max(s, axis=-1, keepdims=True) for s in scores])
            ps = [jnp.exp(s - m) for s in scores]
            l = functools.reduce(jnp.add, [jnp.sum(p, axis=-1, keepdims=True) for p in ps])
            p = jnp.concatenate([p.astype(bf16) for p in ps], axis=-1)

            outs = [None] * nvr
            for r in range(nvr):
                for c in range(nvc):
                    part = consume(t, lambda: jax.lax.dot_general(
                        p[:, c * _V_COLS:(c + 1) * _V_COLS],
                        vbuf[slot, pl.ds(r * _V_ROWS, _V_ROWS), pl.ds(c * _V_COLS, _V_COLS)],
                        (((1,), (1,)), ((), ())), preferred_element_type=f32))
                    outs[r] = part if outs[r] is None else outs[r] + part
                    t += 1
            o = jnp.concatenate(outs, axis=-1)
            o = jnp.where(own_head, o / l, 0.0).astype(bf16)

            acc = acc + consume(t, lambda: jnp.dot(o, wobuf[slot], preferred_element_type=f32))
            assert t == n_pieces - 1
            return acc

        acc = jax.lax.fori_loop(0, n_pairs - 1, body, jnp.zeros((8, d), f32))
        acc = body(n_pairs - 1, acc, last=True)
        a = acc[0:1] + acc[4:5]
        o_ref[0] = (gate * a + mlp_term).astype(o_ref.dtype)

    kt = jnp.transpose(A_k_cache, (0, 1, 3, 2)).reshape(n_pairs, _PR, sk)
    vt = jnp.transpose(A_v_cache, (0, 1, 3, 2)).reshape(n_pairs, _PR, sk)

    return pl.pallas_call(
        kernel_function,
        in_specs=[pl.BlockSpec(memory_space=pl.ANY) for _ in range(10)],
        out_specs=pl.BlockSpec(memory_space=pltpu.VMEM),
        out_shape=jax.ShapeDtypeStruct((batch, sq, d), A_x.dtype),
        scratch_shapes=[
            pltpu.VMEM((batch, sq, d), A_x.dtype),
            pltpu.VMEM((d,), gate_w.dtype),
            pltpu.VMEM((f,), B_b1.dtype),
            pltpu.VMEM((d,), B_b2.dtype),
            pltpu.VMEM((2, _PR, win), A_k_cache.dtype),
            pltpu.VMEM((2, _PR, win), A_v_cache.dtype),
            pltpu.VMEM((2, d, _PR), A_wq.dtype),
            pltpu.VMEM((2, _PR, d), A_wo.dtype),
            pltpu.VMEM((d, f), B_w1.dtype),
            pltpu.VMEM((f, d), B_w2.dtype),
            pltpu.SemaphoreType.DMA((2, nk)),
            pltpu.SemaphoreType.DMA((2, nvr * nvc)),
            pltpu.SemaphoreType.DMA((2, _WQ_PIECES)),
            pltpu.SemaphoreType.DMA((2,)),
            pltpu.SemaphoreType.DMA((4,)),
            pltpu.SemaphoreType.DMA((2, _MLP_PIECES)),
        ],
        compiler_params=pltpu.CompilerParams(vmem_limit_bytes=64 * 1024 * 1024),
    )(A_x, gate_w, B_b1, B_b2, kt, vt, A_wq, A_wo, B_w1, B_w2)
```
